```python
import os as _os
_os.environ.setdefault("JAX_PLATFORMS", "cpu")
import jax
import jax.numpy as jnp

def _softmax(x, axis=-1):
    return jax.nn.softmax(x, axis=axis)
def _gelu(x):
    return jax.nn.gelu(x, approximate=True)
def _silu(x):
    return jax.nn.silu(x)
def _sigmoid(x):
    return jax.nn.sigmoid(x)
def _layernorm(x, axis=-1, eps=1e-5):
    m = jnp.mean(x, axis=axis, keepdims=True)
    v = jnp.var(x, axis=axis, keepdims=True)
    return (x - m) / jnp.sqrt(v + eps)
def _scatter_add(tgt, idx, src, axis=0):
    return tgt.at[idx].add(src)
def _segment_sum(src, seg, n):
    return jax.ops.segment_sum(src, seg, n)
class _Rng:
    def __init__(self, key):
        self._k = key
    def _next(self):
        self._k, sub = jax.random.split(self._k)
        return sub
    def normal(self, shape):
        return jax.random.normal(self._next(), shape, dtype=jnp.bfloat16)
    def randint(self, lo, hi, shape):
        return jax.random.randint(self._next(), shape, lo, hi, dtype=jnp.int32)
    def uniform(self, shape, lo=0.0, hi=1.0):
        return jax.random.uniform(self._next(), shape, jnp.bfloat16, lo, hi)
    def permutation(self, n):
        return jax.random.permutation(self._next(), n)


kernel_name = 'parallel_sum__grouped_kv_mqa__dense_activation_silu__prompt'

def setup_inputs():
    _rng = _Rng(jax.random.key(int.from_bytes(__import__("os").urandom(4), "little")))
    _w = (lambda a: (lambda t: t.astype(jnp.bfloat16) if jnp.issubdtype(t.dtype, jnp.floating) else t)(jnp.asarray(a)))
    def _A_setup():
        B, S, D, H = 1, 2048, 512, 32
        Dh = D // H
        return {
            "x": _w((lambda *s: _rng.normal(s) * 0.05)(B, S, D)),
            "wq": _w((lambda *s: _rng.normal(s) * 0.05)(D, H * Dh)),
            "wk": _w((lambda *s: _rng.normal(s) * 0.05)(D, Dh)),
            "wv": _w((lambda *s: _rng.normal(s) * 0.05)(D, Dh)),
            "wo": _w((lambda *s: _rng.normal(s) * 0.05)(H * Dh, D)),
        }
    _A_in = _A_setup()

    def _B_setup():
        B, S, D, F = 1, 2048, 512, 1376
        return {
            "x": _w((lambda *s: _rng.normal(s) * 0.05)(B, S, D)),
            "w1": _w((lambda *s: _rng.normal(s) * 0.05)(D, F) * (D ** -0.5)),
            "w2": _w((lambda *s: _rng.normal(s) * 0.05)(F, D) * (F ** -0.5)),
        }
    _B_in = _B_setup()

    return {
        "A_x": _A_in["x"],
        "A_wq": _A_in["wq"],
        "A_wk": _A_in["wk"],
        "A_wv": _A_in["wv"],
        "A_wo": _A_in["wo"],
        "B_x": _B_in["x"],
        "B_w1": _B_in["w1"],
        "B_w2": _B_in["w2"],
    }

def reference(A_x, A_wq, A_wk, A_wv, A_wo, B_x, B_w1, B_w2):
    def _A_ref(x, wq, wk, wv, wo):
        B, S, D = x.shape
        H = 32
        Dh = D // H
        q = (lambda x, *d: x.transpose(*d))((x @ wq).reshape(B, S, H, Dh), 0, 2, 1, 3)
        k = x @ wk
        v = x @ wv
        scores = jnp.einsum("bhqd,bkd->bhqk", q, k) * (Dh ** -0.5)
        p = _softmax(scores, axis=-1)
        o = jnp.einsum("bhqk,bkd->bhqd", p, v)
        return (lambda x, *d: x.transpose(*d))(o, 0, 2, 1, 3).reshape(B, S, H * Dh) @ wo

    def _B_ref(x, w1, w2):
        h = jnp.einsum("bsd,df->bsf", x, w1)
        h = _silu(h)
        out = jnp.einsum("bsf,fd->bsd", h, w2)
        return out

    x = A_x
    xn = _layernorm(x, axis=-1)
    return x + _A_ref(xn, A_wq, A_wk, A_wv, A_wo) + _B_ref(xn, B_w1, B_w2)
```

```python
import functools
import jax
import jax.numpy as jnp
from jax import lax
import jax.experimental.pallas as pl
import jax.experimental.pallas.tpu as pltpu

H = 32
DH = 16
EPS = 1e-5
LOG2E = 1.4426950408889634
NT = (((1,), (1,)), ((), ()))
TN = (((0,), (0,)), ((), ()))
f32 = jnp.float32
bf16 = jnp.bfloat16


def make(TQ=128, KC=512, VR=32, RB=256, flags=None, border=0):
    def body(x_hbm, wq_ref, wk_ref, wv_ref, wo_ref, w1_ref, w2_ref, o_ref,
             xn_s, q_s, kt_s, vt_s, ot_s, sa, wo_s, w1_s, w2_s, ob, sem, osem, x_ref, xsem):
        def xcp(i):
            return pltpu.make_async_copy(x_hbm.at[pl.ds(i * RB, RB), :], x_ref.at[pl.ds(i * RB, RB), :], xsem.at[i])
        for i in range(x_ref.shape[0] // RB):
            xcp(i).start()
        cps = [pltpu.make_async_copy(a, b, sem.at[i]) for i, (a, b) in enumerate(((wo_ref, wo_s), (w1_ref, w1_s), (w2_ref, w2_s)))]
        S, D = x_ref.shape
        NQ = S // TQ
        NC = S // KC
        def pro(i, _):
            rows = pl.ds(pl.multiple_of(i * RB, RB), RB)
            xcp(i).wait()

            @pl.when(i == 1)
            def _():
                for cp in cps:
                    cp.start()
            x = x_ref[rows, :].astype(f32)
            m = jnp.mean(x, axis=-1, keepdims=True)
            xc = x - m
            v = jnp.mean(xc * xc, axis=-1, keepdims=True)
            xn = (xc * lax.rsqrt(v + EPS)).astype(bf16)
            xn_s[rows, :] = xn
            q = jnp.dot(xn, wq_ref[...], preferred_element_type=f32) * (DH ** -0.5 * LOG2E)
            q_s[:, rows] = q.T.astype(bf16)
            kt_s[rows, :] = lax.dot_general(xn, wk_ref[...], NT, preferred_element_type=f32).astype(bf16)
            vt = lax.dot_general(wv_ref[...], xn, NT, preferred_element_type=f32)
            vt_s[:, rows] = vt.astype(bf16)
            return 0
        lax.fori_loop(0, S // RB, pro, 0)

        def get_q(u):
            return q_s[pl.ds(pl.multiple_of((u % H) * DH, DH), DH), pl.ds(pl.multiple_of((u // H) * TQ, TQ), TQ)]

        def step(u, m_cur, s_cur, s_nxt, do_a=True, do_b=True):
            if do_a:
                qm = get_q(u + 1)
            mx = None
            acc = None
            l = None
            for ci in range(NC):
                ks = slice(ci * KC, (ci + 1) * KC)
                if do_b:
                    sc = s_cur[ks, :]
                if do_a:
                    s = jnp.dot(kt_s[ks, :], qm, preferred_element_type=f32)
                    s_nxt[ks, :] = s
                    cm = jnp.max(s.reshape(KC // 8, 8, TQ), axis=0)
                    mx = cm if mx is None else jnp.maximum(mx, cm)
                if do_b:
                    p = jnp.exp2(sc - m_cur)
                    if VR == DH:
                        cl = jnp.sum(p.reshape(KC // 8, 8, TQ), axis=0)
                        l = cl if l is None else l + cl
                    pv = jnp.dot(vt_s[:, ks], p.astype(bf16), preferred_element_type=f32)
                    acc = pv if acc is None else acc + pv
            if do_b:
                if VR == DH:
                    den = jnp.sum(l, axis=0, keepdims=True)
                else:
                    den = acc[DH:DH + 1]
                o = acc[:DH] / den
                qb = u // H
                h = u % H
                ot_s[qb, pl.ds(pl.multiple_of(h * DH, DH), DH), :] = o.astype(bf16)
            if do_a:
                return jnp.max(mx, axis=0, keepdims=True)
            return m_cur

        NU = NQ * H
        m0 = step(-1, None, None, sa, do_b=False)

        if border == 1:
            m = lax.fori_loop(0, NU - 2, lambda u, m: step(u, m, sa, sa), m0, unroll=2)
            m = step(NU - 2, m, sa, sa)
        else:
            m = lax.fori_loop(0, NU - 1, lambda u, m: step(u, m, sa, sa), m0)
        step(NU - 1, m, sa, sa, do_a=False)

        for cp in cps:
            cp.wait()

        def ocp(i):
            rows = pl.ds(i * TQ, TQ)
            return pltpu.make_async_copy(ob.at[rows, :], o_ref.at[rows, :], osem.at[i])

        def epi(i, _):
            rows = pl.ds(pl.multiple_of(i * TQ, TQ), TQ)
            xn = xn_s[rows, :]
            hh = lax.dot_general(xn, w1_s[...], NT, preferred_element_type=f32)
            hf = 0.5 * hh; hh = (hf * jnp.tanh(hf) + hf).astype(bf16)
            y = jnp.dot(hh, w2_s[...], preferred_element_type=f32)
            y = y + lax.dot_general(ot_s[i], wo_s[...], TN, preferred_element_type=f32)
            ob[rows, :] = (y + x_ref[rows, :].astype(f32)).astype(ob.dtype)
            ocp(i).start()
            return 0
        lax.fori_loop(0, NQ, epi, 0)
        for i in range(NQ):
            ocp(i).wait()

    @jax.jit
    def fn(A_x, A_wq, A_wk, A_wv, A_wo, B_x, B_w1, B_w2):
        B, S, D = A_x.shape
        x = A_x.reshape(S, D)
        out = pl.pallas_call(
            body,
            out_shape=jax.ShapeDtypeStruct((S, D), A_x.dtype),
            in_specs=[pl.BlockSpec(memory_space=pl.ANY)] + [pl.BlockSpec(memory_space=pltpu.VMEM)] * 3 + [pl.BlockSpec(memory_space=pl.ANY)] * 3,
            out_specs=pl.BlockSpec(memory_space=pl.ANY),
            scratch_shapes=[
                pltpu.VMEM((S, D), bf16), pltpu.VMEM((D, S), bf16),
                pltpu.VMEM((S, DH), bf16), pltpu.VMEM((VR, S), bf16),
                pltpu.VMEM((S // TQ, D, TQ), bf16),
                pltpu.VMEM((S, TQ), f32),
                pltpu.VMEM(A_wo.shape, bf16), pltpu.VMEM(B_w2.shape, bf16), pltpu.VMEM(B_w2.shape, bf16),
                pltpu.VMEM((S, D), A_x.dtype), pltpu.SemaphoreType.DMA((3,)), pltpu.SemaphoreType.DMA((S // TQ,)),
                pltpu.VMEM((S, D), A_x.dtype), pltpu.SemaphoreType.DMA((S // RB,)),
            ],
            compiler_params=pltpu.CompilerParams(vmem_limit_bytes=100 * 1024 * 1024, flags=flags),
            name="fused",
        )(x, A_wq, A_wk.T, A_wv.T, A_wo, B_w1.T, B_w2)
        return out.reshape(B, S, D)
    return fn


pallas_parallel_sum__grouped_kv_mqa__dense_activation_silu__prompt_kernel = make(TQ=512,KC=128,VR=16,RB=512)
```
